```python
import os as _os
_os.environ.setdefault("JAX_PLATFORMS", "cpu")
import jax
import jax.numpy as jnp

def _softmax(x, axis=-1):
    return jax.nn.softmax(x, axis=axis)
def _gelu(x):
    return jax.nn.gelu(x, approximate=True)
def _silu(x):
    return jax.nn.silu(x)
def _sigmoid(x):
    return jax.nn.sigmoid(x)
def _layernorm(x, axis=-1, eps=1e-5):
    m = jnp.mean(x, axis=axis, keepdims=True)
    v = jnp.var(x, axis=axis, keepdims=True)
    return (x - m) / jnp.sqrt(v + eps)
def _scatter_add(tgt, idx, src, axis=0):
    return tgt.at[idx].add(src)
def _segment_sum(src, seg, n):
    return jax.ops.segment_sum(src, seg, n)
class _Rng:
    def __init__(self, key):
        self._k = key
    def _next(self):
        self._k, sub = jax.random.split(self._k)
        return sub
    def normal(self, shape):
        return jax.random.normal(self._next(), shape, dtype=jnp.bfloat16)
    def randint(self, lo, hi, shape):
        return jax.random.randint(self._next(), shape, lo, hi, dtype=jnp.int32)
    def uniform(self, shape, lo=0.0, hi=1.0):
        return jax.random.uniform(self._next(), shape, jnp.bfloat16, lo, hi)
    def permutation(self, n):
        return jax.random.permutation(self._next(), n)


kernel_name = 'concat_heads__mha_block_cached__mha_block_cached__near_ridge'

def setup_inputs():
    _rng = _Rng(jax.random.key(int.from_bytes(__import__("os").urandom(4), "little")))
    _w = (lambda a: (lambda t: t.astype(jnp.bfloat16) if jnp.issubdtype(t.dtype, jnp.floating) else t)(jnp.asarray(a)))
    def _A_setup():
        B, Sq, D = 8, 160, 512
        H, Sk, Dh = 32, 512, 128
        return {
            "x": _w((lambda *s: _rng.normal(s) * 0.8)(B, Sq, D)),
            "k_cache": _w((lambda *s: _rng.normal(s) * 0.8)(B, H, Sk, Dh)),
            "v_cache": _w((lambda *s: _rng.normal(s) * 0.05)(B, H, Sk, Dh)),
            "wq": _w((lambda *s: _rng.normal(s) * 0.8)(D, H * Dh) * (D ** -0.5)),
            "wo": _w((lambda *s: _rng.normal(s) * 0.05)(H * Dh, D) * ((H * Dh) ** -0.5)),
        }
    _A_in = _A_setup()

    def _B_setup():
        B, Sq, D = 8, 160, 512
        H, Sk, Dh = 32, 512, 128
        return {
            "x": _w((lambda *s: _rng.normal(s) * 0.8)(B, Sq, D)),
            "k_cache": _w((lambda *s: _rng.normal(s) * 0.8)(B, H, Sk, Dh)),
            "v_cache": _w((lambda *s: _rng.normal(s) * 0.05)(B, H, Sk, Dh)),
            "wq": _w((lambda *s: _rng.normal(s) * 0.8)(D, H * Dh) * (D ** -0.5)),
            "wo": _w((lambda *s: _rng.normal(s) * 0.05)(H * Dh, D) * ((H * Dh) ** -0.5)),
        }
    _B_in = _B_setup()

    return {
        "A_x": _A_in["x"],
        "A_k_cache": _A_in["k_cache"],
        "A_v_cache": _A_in["v_cache"],
        "A_wq": _A_in["wq"],
        "A_wo": _A_in["wo"],
        "B_x": _B_in["x"],
        "B_k_cache": _B_in["k_cache"],
        "B_v_cache": _B_in["v_cache"],
        "B_wq": _B_in["wq"],
        "B_wo": _B_in["wo"],
    }

def reference(A_x, A_k_cache, A_v_cache, A_wq, A_wo, B_x, B_k_cache, B_v_cache, B_wq, B_wo):
    def _A_ref(x, k_cache, v_cache, wq, wo):
        B, Sq, D = x.shape
        H, Dh = 32, 128
        q = (lambda x, *d: x.transpose(*d))((x @ wq).reshape(B, Sq, H, Dh), 0, 2, 1, 3)
        scores = jnp.einsum("bhqd,bhkd->bhqk", q, k_cache) * (Dh ** -0.5)
        p = _softmax(scores, axis=-1)
        o = jnp.einsum("bhqk,bhkd->bhqd", p, v_cache)
        return (lambda x, *d: x.transpose(*d))(o, 0, 2, 1, 3).reshape(B, Sq, H * Dh) @ wo

    def _B_ref(x, k_cache, v_cache, wq, wo):
        B, Sq, D = x.shape
        H, Dh = 32, 128
        q = (lambda x, *d: x.transpose(*d))((x @ wq).reshape(B, Sq, H, Dh), 0, 2, 1, 3)
        scores = jnp.einsum("bhqd,bhkd->bhqk", q, k_cache) * (Dh ** -0.5)
        p = _softmax(scores, axis=-1)
        o = jnp.einsum("bhqk,bhkd->bhqd", p, v_cache)
        return (lambda x, *d: x.transpose(*d))(o, 0, 2, 1, 3).reshape(B, Sq, H * Dh) @ wo

    a = _A_ref(A_x, A_k_cache, A_v_cache, A_wq, A_wo)
    b = _B_ref(B_x, B_k_cache, B_v_cache, B_wq, B_wo)
    return jnp.concatenate([a, b], axis=-1)
```

```python
import functools

import jax
import jax.numpy as jnp
from jax import lax
import jax.experimental.pallas as pl
import jax.experimental.pallas.tpu as pltpu


HG = 8
NB = 8


def _kernel(xa_hbm, ka_hbm, va_hbm, wqa_hbm, woa_hbm,
            xb_hbm, kb_hbm, vb_hbm, wqb_hbm, wob_hbm,
            out_hbm,
            xbuf, kbuf, vbuf, wqbuf, wobuf, acc_ref, obuf, qbuf,
            x_sem, wq_sem, wo_sem, kv_sem, o_sem,
            *, nb, sq, d_model, n_heads, sk, dh, hg):
    G = n_heads // hg
    T = G * nb
    lb = nb.bit_length() - 1
    assert nb == 1 << lb and G >= 2 and T >= NB
    scale = dh ** -0.5
    hd = hg * dh
    x_hbm = (xa_hbm, xb_hbm)
    k_hbm = (ka_hbm, kb_hbm)
    v_hbm = (va_hbm, vb_hbm)
    wq_hbm = (wqa_hbm, wqb_hbm)
    wo_hbm = (woa_hbm, wob_hbm)

    def kv_copies(t):
        slot = t & (NB - 1)
        g = t >> lb
        b = t & (nb - 1)
        cps = []
        for br in range(2):
            cps.append(pltpu.make_async_copy(
                k_hbm[br].at[b, pl.ds(g * hg, hg)], kbuf.at[slot, br],
                kv_sem.at[slot, 2 * br]))
            cps.append(pltpu.make_async_copy(
                v_hbm[br].at[b, pl.ds(g * hg, hg)], vbuf.at[slot, br],
                kv_sem.at[slot, 2 * br + 1]))
        return cps

    def wq_copy(br, g):
        return pltpu.make_async_copy(
            wq_hbm[br].at[:, pl.ds(g * hd, hd)], wqbuf.at[br, g],
            wq_sem.at[br, g])

    def wo_copy(br):
        return pltpu.make_async_copy(wo_hbm[br], wobuf.at[br], wo_sem.at[br])

    def x_copy(br):
        return pltpu.make_async_copy(x_hbm[br], xbuf.at[br], x_sem.at[br])

    def out_copy(b):
        return pltpu.make_async_copy(obuf.at[b], out_hbm.at[b], o_sem.at[b])

    pieces = [(br, g) for g in range(G) for br in range(2)]
    batches = [
        [x_copy(1), wq_copy(1, 0)] + [wq_copy(br, 1) for br in range(2)],
        [wq_copy(br, g) for g in range(2, G) for br in range(2)],
    ]
    batches.append(kv_copies(0) + [wo_copy(0)])
    batches.append(kv_copies(1) + [wo_copy(1)])
    rest = [kv_copies(u) for u in range(2, NB - 1)]
    n_left = len(pieces) - len(batches)
    for i in range(n_left):
        take = -(-len(rest) // (n_left - i))
        batches.append([cp for grp in rest[:take] for cp in grp])
        rest = rest[take:]

    x_copy(0).start()
    wq_copy(0, 0).start()
    acc_ref[...] = jnp.zeros(acc_ref.shape, acc_ref.dtype)
    for i, (br, g) in enumerate(pieces):
        if g == 0:
            x_copy(br).wait()
        wq_copy(br, g).wait()
        for cp in batches[i]:
            cp.start()
        xall = xbuf[br].reshape(nb * sq, d_model)
        q = jnp.dot(xall, wqbuf[br, g], preferred_element_type=jnp.float32)
        qbuf[g, :, br] = (q * scale).astype(jnp.bfloat16).reshape(nb, sq, hd)
    for br in range(2):
        wo_copy(br).wait()

    def make_body(last):
        def body(t, carry):
            g = t >> lb
            b = t & (nb - 1)
            slot = t & (NB - 1)

            for cp in kv_copies(t):
                cp.wait()

            @pl.when(t + NB - 1 < T)
            def _():
                for cp in kv_copies(t + NB - 1):
                    cp.start()

            def qk(br, h):
                qh = qbuf[g, b, br, :, h * dh:(h + 1) * dh]
                return lax.dot_general(qh, kbuf[slot, br, h],
                                       (((1,), (1,)), ((), ())),
                                       preferred_element_type=jnp.float32)

            def sm_pv(s, br, h):
                m = jnp.max(s, axis=-1, keepdims=True)
                p = jnp.exp(s - m)
                l = jnp.sum(p, axis=-1, keepdims=True)
                o = jnp.dot(p.astype(jnp.bfloat16), vbuf[slot, br, h],
                            preferred_element_type=jnp.float32)
                r = pl.reciprocal(l, approx=True)
                r = r * (2.0 - l * r)
                return (o * r).astype(jnp.bfloat16)

            items = [(br, h) for h in range(hg) for br in range(2)]
            outs = []
            s_next = qk(*items[0])
            for i, (br, h) in enumerate(items):
                s_cur = s_next
                if i + 1 < len(items):
                    s_next = qk(*items[i + 1])
                outs.append(sm_pv(s_cur, br, h))
            for br in range(2):
                o_all = jnp.concatenate(outs[br::2], axis=-1)
                wo = wobuf[br, pl.ds(pl.multiple_of(g * hd, hd), hd), :]
                c = jnp.dot(o_all, wo, preferred_element_type=jnp.float32)
                sl = slice(br * d_model, (br + 1) * d_model)
                n = acc_ref[b, :, sl] + c
                if last:
                    obuf[b, :, sl] = n.astype(obuf.dtype)
                else:
                    acc_ref[b, :, sl] = n

            if last:
                out_copy(b).start()
            return carry
        return body

    with jax.named_scope("loop1"):
        lax.fori_loop(0, T - nb, make_body(False), 0)
    with jax.named_scope("loop2"):
        lax.fori_loop(T - nb, T, make_body(True), 0)

    for b in range(nb):
        out_copy(b).wait()


@jax.jit
def pallas_concat_heads__mha_block_cached__mha_block_cached__near_ridge_kernel(
    A_x, A_k_cache, A_v_cache, A_wq, A_wo, B_x, B_k_cache, B_v_cache, B_wq, B_wo,
):
    B, Sq, D = A_x.shape
    _, H, Sk, Dh = A_k_cache.shape
    hg = HG
    G = H // hg
    dt = A_x.dtype
    any_spec = pl.BlockSpec(memory_space=pl.ANY)
    kern = functools.partial(_kernel, nb=B, sq=Sq, d_model=D, n_heads=H, sk=Sk,
                             dh=Dh, hg=hg)
    return pl.pallas_call(
        kern,
        in_specs=[any_spec] * 10,
        out_specs=any_spec,
        out_shape=jax.ShapeDtypeStruct((B, Sq, 2 * D), dt),
        scratch_shapes=[
            pltpu.VMEM((2, B, Sq, D), dt),
            pltpu.VMEM((NB, 2, hg, Sk, Dh), dt),
            pltpu.VMEM((NB, 2, hg, Sk, Dh), dt),
            pltpu.VMEM((2, G, D, hg * Dh), dt),
            pltpu.VMEM((2, H * Dh, D), dt),
            pltpu.VMEM((B, Sq, 2 * D), jnp.float32),
            pltpu.VMEM((B, Sq, 2 * D), dt),
            pltpu.VMEM((G, B, 2, Sq, hg * Dh), dt),
            pltpu.SemaphoreType.DMA((2,)),
            pltpu.SemaphoreType.DMA((2, G)),
            pltpu.SemaphoreType.DMA((2,)),
            pltpu.SemaphoreType.DMA((NB, 4)),
            pltpu.SemaphoreType.DMA((B,)),
        ],
        compiler_params=pltpu.CompilerParams(
            vmem_limit_bytes=110 * 1024 * 1024,
            disable_bounds_checks=True,
        ),
    )(A_x, A_k_cache, A_v_cache, A_wq, A_wo,
      B_x, B_k_cache, B_v_cache, B_wq, B_wo)
```

```python
import functools
import math

import jax
import jax.numpy as jnp
from jax import lax
import jax.experimental.pallas as pl
import jax.experimental.pallas.tpu as pltpu


HG = 8
NB = 8
UNROLL = 2
NF = 2


def _kernel(xa_hbm, ka_hbm, va_hbm, wqa_hbm, woa_hbm,
            xb_hbm, kb_hbm, vb_hbm, wqb_hbm, wob_hbm,
            out_hbm,
            xbuf, kbuf, vbuf, wqbuf, wobuf, acc_ref, obuf, qbuf,
            x_sem, wq_sem, wo_sem, kv_sem, o_sem,
            *, nb, sq, d_model, n_heads, dh, hg):
    G = n_heads // hg
    T = G * nb
    lb = nb.bit_length() - 1
    assert nb == 1 << lb and G >= 2 and T >= NB and nb % UNROLL == 0
    scale = dh ** -0.5 * math.log2(math.e)
    hd = hg * dh
    x_hbm = (xa_hbm, xb_hbm)
    k_hbm = (ka_hbm, kb_hbm)
    v_hbm = (va_hbm, vb_hbm)
    wq_hbm = (wqa_hbm, wqb_hbm)
    wo_hbm = (woa_hbm, wob_hbm)

    def kv_copies(t):
        slot = t & (NB - 1)
        g = t >> lb
        b = t & (nb - 1)
        cps = []
        for br in range(2):
            cps.append(pltpu.make_async_copy(
                k_hbm[br].at[b, pl.ds(g * hg, hg)], kbuf.at[slot, br],
                kv_sem.at[slot, 2 * br]))
            cps.append(pltpu.make_async_copy(
                v_hbm[br].at[b, pl.ds(g * hg, hg)], vbuf.at[slot, br],
                kv_sem.at[slot, 2 * br + 1]))
        return cps

    def wq_copy(br, g):
        return pltpu.make_async_copy(
            wq_hbm[br].at[:, pl.ds(g * hd, hd)], wqbuf.at[br, g],
            wq_sem.at[br, g])

    def wo_copy(br):
        return pltpu.make_async_copy(wo_hbm[br], wobuf.at[br], wo_sem.at[br])

    def xa_first():
        return pltpu.make_async_copy(x_hbm[0].at[pl.ds(0, NF)],
                                     xbuf.at[0, pl.ds(0, NF)], x_sem.at[2])

    def xa_rest():
        return pltpu.make_async_copy(x_hbm[0].at[pl.ds(NF, nb - NF)],
                                     xbuf.at[0, pl.ds(NF, nb - NF)],
                                     x_sem.at[0])

    def xb_copy():
        return pltpu.make_async_copy(x_hbm[1], xbuf.at[1], x_sem.at[1])

    def out_copy(b):
        return pltpu.make_async_copy(obuf.at[b], out_hbm.at[b], o_sem.at[b])

    def qproj(br, g, b0, b1):
        n = b1 - b0
        xall = xbuf[br, b0:b1].reshape(n * sq, d_model)
        q = jnp.dot(xall, wqbuf[br, g], preferred_element_type=jnp.float32)
        qbuf[g, b0:b1, br] = (q * scale).astype(qbuf.dtype).reshape(n, sq, hd)

    pieces = [(br, g) for br in range(2) for g in range(G)]
    batches = [
        [wq_copy(0, g) for g in range(1, G)] + [xb_copy()],
        [wq_copy(1, g) for g in range(G)],
        kv_copies(0) + [wo_copy(0)],
        kv_copies(1) + [wo_copy(1)],
    ]
    rest = [kv_copies(u) for u in range(2, NB - UNROLL)]
    n_left = len(pieces) - len(batches)
    assert n_left >= 1
    for i in range(n_left):
        take = -(-len(rest) // (n_left - i))
        batches.append([cp for grp in rest[:take] for cp in grp])
        rest = rest[take:]

    xa_first().start()
    wq_copy(0, 0).start()
    acc_ref[...] = jnp.zeros(acc_ref.shape, acc_ref.dtype)
    xa_first().wait()
    wq_copy(0, 0).wait()
    xa_rest().start()
    qproj(0, 0, 0, NF)
    for i, (br, g) in enumerate(pieces):
        if i == 0:
            xa_rest().wait()
        elif i == 1:
            for g2 in range(1, G):
                wq_copy(0, g2).wait()
        elif i == G:
            xb_copy().wait()
            for g2 in range(G):
                wq_copy(1, g2).wait()
        for cp in batches[i]:
            cp.start()
        qproj(br, g, NF if i == 0 else 0, nb)
    for br in range(2):
        wo_copy(br).wait()

    def make_body(last):
        def step(t):
            g = t >> lb
            b = t & (nb - 1)
            slot = t & (NB - 1)

            def qk(br, h):
                qh = qbuf[g, b, br, :, h * dh:(h + 1) * dh]
                return lax.dot_general(qh, kbuf[slot, br, h],
                                       (((1,), (1,)), ((), ())),
                                       preferred_element_type=jnp.float32)

            def sm_pv(s, br, h):
                m = jnp.max(s, axis=-1, keepdims=True)
                p = jnp.exp2(s - m)
                l = jnp.sum(p, axis=-1, keepdims=True)
                o = jnp.dot(p.astype(vbuf.dtype), vbuf[slot, br, h],
                            preferred_element_type=jnp.float32)
                r = pl.reciprocal(l, approx=True)
                r = r * (2.0 - l * r)
                return (o * r).astype(wobuf.dtype)

            items = [(br, h) for h in range(hg) for br in range(2)]
            outs = []
            s_next = qk(*items[0])
            for i, (br, h) in enumerate(items):
                s_cur = s_next
                if i + 1 < len(items):
                    s_next = qk(*items[i + 1])
                outs.append(sm_pv(s_cur, br, h))
            for br in range(2):
                o_all = jnp.concatenate(outs[br::2], axis=-1)
                wo = wobuf[br, pl.ds(pl.multiple_of(g * hd, hd), hd), :]
                c = jnp.dot(o_all, wo, preferred_element_type=jnp.float32)
                sl = slice(br * d_model, (br + 1) * d_model)
                n = acc_ref[b, :, sl] + c
                if last:
                    obuf[b, :, sl] = n.astype(obuf.dtype)
                else:
                    acc_ref[b, :, sl] = n

        def body(tt, carry):
            t0 = tt * UNROLL
            for u in range(UNROLL):
                for cp in kv_copies(t0 + u):
                    cp.wait()

            @pl.when(t0 + NB <= T)
            def _():
                for u in range(UNROLL):
                    for cp in kv_copies(t0 + u + NB - UNROLL):
                        cp.start()

            for u in range(UNROLL):
                step(t0 + u)
                if last:
                    out_copy((t0 + u) & (nb - 1)).start()
            return carry

        return body

    lax.fori_loop(0, (T - nb) // UNROLL, make_body(False), 0)
    lax.fori_loop((T - nb) // UNROLL, T // UNROLL, make_body(True), 0)

    for b in range(nb):
        out_copy(b).wait()


@jax.jit
def pallas_concat_heads__mha_block_cached__mha_block_cached__near_ridge_kernel(
    A_x: jax.Array,
    A_k_cache: jax.Array,
    A_v_cache: jax.Array,
    A_wq: jax.Array,
    A_wo: jax.Array,
    B_x: jax.Array,
    B_k_cache: jax.Array,
    B_v_cache: jax.Array,
    B_wq: jax.Array,
    B_wo: jax.Array,
):
    B, Sq, D = A_x.shape
    _, H, Sk, Dh = A_k_cache.shape
    hg = HG
    G = H // hg
    dt = A_x.dtype
    any_spec = pl.BlockSpec(memory_space=pl.ANY)
    kern = functools.partial(_kernel, nb=B, sq=Sq, d_model=D, n_heads=H,
                             dh=Dh, hg=hg)
    return pl.pallas_call(
        kern,
        in_specs=[any_spec] * 10,
        out_specs=any_spec,
        out_shape=jax.ShapeDtypeStruct((B, Sq, 2 * D), dt),
        scratch_shapes=[
            pltpu.VMEM((2, B, Sq, D), dt),
            pltpu.VMEM((NB, 2, hg, Sk, Dh), dt),
            pltpu.VMEM((NB, 2, hg, Sk, Dh), dt),
            pltpu.VMEM((2, G, D, hg * Dh), dt),
            pltpu.VMEM((2, H * Dh, D), dt),
            pltpu.VMEM((B, Sq, 2 * D), jnp.float32),
            pltpu.VMEM((B, Sq, 2 * D), dt),
            pltpu.VMEM((G, B, 2, Sq, hg * Dh), dt),
            pltpu.SemaphoreType.DMA((3,)),
            pltpu.SemaphoreType.DMA((2, G)),
            pltpu.SemaphoreType.DMA((2,)),
            pltpu.SemaphoreType.DMA((NB, 4)),
            pltpu.SemaphoreType.DMA((B,)),
        ],
        compiler_params=pltpu.CompilerParams(
            vmem_limit_bytes=110 * 1024 * 1024,
            disable_bounds_checks=True,
        ),
    )(A_x, A_k_cache, A_v_cache, A_wq, A_wo,
      B_x, B_k_cache, B_v_cache, B_wq, B_wo)
```
